```python
import os as _os
_os.environ.setdefault('JAX_PLATFORMS', 'cpu')
import jax
import jax.numpy as jnp

def _softmax(x, axis=-1):
    return jax.nn.softmax(x, axis=axis)

def _gelu(x):
    return jax.nn.gelu(x, approximate=True)

def _silu(x):
    return jax.nn.silu(x)

def _sigmoid(x):
    return jax.nn.sigmoid(x)

def _layernorm(x, axis=-1, eps=1e-05):
    m = jnp.mean(x, axis=axis, keepdims=True)
    v = jnp.var(x, axis=axis, keepdims=True)
    return (x - m) / jnp.sqrt(v + eps)

def _scatter_add(tgt, idx, src, axis=0):
    return tgt.at[idx].add(src)

def _segment_sum(src, seg, n):
    return jax.ops.segment_sum(src, seg, n)

class _Rng:

    def __init__(self, key):
        self._k = key

    def _next(self):
        self._k, sub = jax.random.split(self._k)
        return sub

    def normal(self, shape):
        return jax.random.normal(self._next(), shape, dtype=jnp.bfloat16)

    def randint(self, lo, hi, shape):
        return jax.random.randint(self._next(), shape, lo, hi, dtype=jnp.int32)

    def uniform(self, shape, lo=0.0, hi=1.0):
        return jax.random.uniform(self._next(), shape, jnp.bfloat16, lo, hi)

    def permutation(self, n):
        return jax.random.permutation(self._next(), n)
kernel_name = 'sequential_preLN__linear_attn_block__mixer_gmlp__prompt'

def setup_inputs():
    _rng = _Rng(jax.random.key(int.from_bytes(__import__("os").urandom(4), "little")))
    _w = lambda a: (lambda t: t.astype(jnp.bfloat16) if jnp.issubdtype(t.dtype, jnp.floating) else t)(jnp.asarray(a))

    def _A_setup():
        B, S, D = (1, 2048, 512)
        return {'x': _w((lambda *s: _rng.normal(s) * 0.05)(B, S, D)), 'wqkv': _w((lambda *s: _rng.normal(s) * 0.05)(D, 3 * D)), 'wo': _w((lambda *s: _rng.normal(s) * 0.05)(D, D))}
    _A_in = _A_setup()

    def _B_setup():
        B, S, D, F = (1, 2048, 512, 1792)
        Fh = F // 2
        return {'x': _w((lambda *s: _rng.normal(s) * 0.05)(B, S, D)), 'w_in': _w((lambda *s: _rng.normal(s) * 0.4)(D, 2 * Fh)), 'w_sp': _w(0.01 * (lambda *s: _rng.normal(s) * 0.4)(S, S)), 'b_sp': _w(1.0 + 0.01 * (lambda *s: _rng.normal(s) * 0.05)(S)), 'w_out': _w((lambda *s: _rng.normal(s) * 0.05)(Fh, D))}
    _B_in = _B_setup()
    return {'A_x': _A_in['x'], 'A_wqkv': _A_in['wqkv'], 'A_wo': _A_in['wo'], 'B_x': _B_in['x'], 'B_w_in': _B_in['w_in'], 'B_w_sp': _B_in['w_sp'], 'B_b_sp': _B_in['b_sp'], 'B_w_out': _B_in['w_out']}

def reference(A_x, A_wqkv, A_wo, B_x, B_w_in, B_w_sp, B_b_sp, B_w_out):

    def _A_ref(x, wqkv, wo):
        B, S, D = x.shape
        H = 32
        Dh = D // H
        qkv = (lambda x, *d: x.transpose(*d))((x @ wqkv).reshape(B, S, 3, H, Dh), 2, 0, 3, 1, 4)
        q, k, v = (qkv[0], qkv[1], qkv[2])
        phi = lambda t: jnp.where(t > 0, t + 1, jnp.exp(t)) + 1e-06
        pq, pk = (phi(q), phi(k))
        kv = jnp.einsum('bhsd,bhse->bhde', pk, v)
        z = jnp.einsum('bhsd->bhd', pk)
        num = jnp.einsum('bhqd,bhde->bhqe', pq, kv)
        den = jnp.einsum('bhqd,bhd->bhq', pq, z)[..., None] + 1e-06
        o = num / den
        return (lambda x, *d: x.transpose(*d))(o, 0, 2, 1, 3).reshape(B, S, D) @ wo

    def _B_ref(x, w_in, w_sp, b_sp, w_out):
        B, S, D = x.shape
        F = w_in.shape[-1]
        Fh = F // 2
        z = _gelu(jnp.einsum('bsd,df->bsf', x, w_in))
        z1 = z[..., :Fh].copy()
        z2 = _layernorm(z[..., Fh:], axis=-1)
        g = jnp.einsum('ts,bsf->btf', w_sp, z2) + b_sp[None, :, None]
        return jnp.einsum('bsf,fd->bsd', z1 * g, w_out)
    x = A_x
    h = x + _A_ref(_layernorm(x, axis=-1), A_wqkv, A_wo)
    h2 = h + _B_ref(_layernorm(h, axis=-1), B_w_in, B_w_sp, B_b_sp, B_w_out)
    return h2
```

```python
import functools
import jax
import jax.numpy as jnp
import numpy as np
from jax import lax
import jax.experimental.pallas as pl
import jax.experimental.pallas.tpu as pltpu

S, D, H, DH, FH = 2048, 512, 32, 16, 896
EPS = 1e-5
F32, BF16 = jnp.float32, jnp.bfloat16


def _ln(x):
    m = jnp.mean(x, axis=-1, keepdims=True)
    d = x - m
    v = jnp.mean(d * d, axis=-1, keepdims=True)
    return d * lax.rsqrt(v + EPS)


def _phi(t):
    return jnp.where(t > 0, t + 1.0, jnp.exp(t)) + 1e-6


def _gelu(x):
    c = np.float32(np.sqrt(2.0 / np.pi))
    return 0.5 * x * (1.0 + jnp.tanh(c * (x + 0.044715 * (x * x * x))))


def _dot(a, b):
    return jnp.dot(a, b, preferred_element_type=F32)


def make_kernel(TM):
    NT = S // TM

    def kernel(x_hbm, wqkv_hbm, wo_hbm, win_hbm, wsp_hbm, bsp_ref, wout_hbm, out_hbm,
               x_v, wqkv_v, wo_v, win_v, wsp_v, wout_v,
               xln_v, h_v, hln_v, z2_v, kv_v, z_v, wp_v, zm_v, out_v, bcol_v, sems, osems):
        cps = [
            pltpu.make_async_copy(x_hbm, x_v, sems.at[0]),
            pltpu.make_async_copy(wqkv_hbm, wqkv_v, sems.at[1]),
            pltpu.make_async_copy(wo_hbm, wo_v, sems.at[2]),
            pltpu.make_async_copy(win_hbm, win_v, sems.at[3]),
            pltpu.make_async_copy(wsp_hbm, wsp_v, sems.at[4]),
            pltpu.make_async_copy(wout_hbm, wout_v, sems.at[5]),
        ]
        for c in cps:
            c.start()
        brow = bsp_ref[...].astype(F32)
        for j in range(S // 128):
            bcol_v[j * 128:(j + 1) * 128, :] = jnp.broadcast_to(brow[j:j + 1, :], (128, 128)).T
        cps[0].wait()
        cps[1].wait()

        kv_v[...] = jnp.zeros_like(kv_v)
        z_v[...] = jnp.zeros_like(z_v)

        def p1(i, _):
            r = pl.ds(pl.multiple_of(i * TM, TM), TM)
            xl = _ln(x_v[r, :].astype(F32)).astype(BF16)
            xln_v[r, :] = xl
            k = _dot(xl, wqkv_v[:, D:2 * D])
            v = _dot(xl, wqkv_v[:, 2 * D:3 * D]).astype(BF16)
            pk = _phi(k)
            z_v[...] += jnp.sum(pk.reshape(TM // 8, 8, D), axis=0)
            pkb = pk.astype(BF16)
            for b in range(4):
                c = slice(b * 128, (b + 1) * 128)
                kv_v[b] += lax.dot_general(pkb[:, c], v[:, c], (((0,), (0,)), ((), ())),
                                           preferred_element_type=F32)
            return 0

        lax.fori_loop(0, NT, p1, 0)

        cps[2].wait()
        ri = lax.broadcasted_iota(jnp.int32, (128, 128), 0) // DH
        ci = lax.broadcasted_iota(jnp.int32, (128, 128), 1) // DH
        mask = ri == ci
        zrow = jnp.sum(z_v[...], axis=0, keepdims=True)
        for b in range(4):
            c = slice(b * 128, (b + 1) * 128)
            kvb = jnp.where(mask, kv_v[b], 0.0).astype(BF16)
            wp_v[c, :] = _dot(kvb, wo_v[c, :]).astype(BF16)
            zm_v[b] = jnp.where(mask, jnp.broadcast_to(zrow[:, c], (128, 128)), 0.0).astype(BF16)

        cps[3].wait()

        def p2(i, _):
            r = pl.ds(pl.multiple_of(i * TM, TM), TM)
            xl = xln_v[r, :]
            q = _dot(xl, wqkv_v[:, 0:D])
            pq = _phi(q)
            pqb = pq.astype(BF16)
            dens = []
            for b in range(4):
                c = slice(b * 128, (b + 1) * 128)
                dens.append(lax.dot_general(pqb[:, c], zm_v[b], (((1,), (1,)), ((), ())),
                                            preferred_element_type=F32))
            den = jnp.concatenate(dens, axis=1) + 1e-6
            o = (pq / den).astype(BF16)
            h = x_v[r, :].astype(F32) + _dot(o, wp_v[...])
            h_v[r, :] = h
            hl = _ln(h).astype(BF16)
            hln_v[r, :] = hl
            z2 = _gelu(_dot(hl, win_v[:, FH:]))
            z2_v[r, :] = _ln(z2).astype(BF16)
            return 0

        lax.fori_loop(0, NT, p2, 0)

        cps[4].wait()
        cps[5].wait()

        def p3(i, _):
            r = pl.ds(pl.multiple_of(i * TM, TM), TM)
            slot = i % 2

            @pl.when(i >= 2)
            def _():
                pltpu.make_async_copy(out_v.at[slot], out_hbm.at[r], osems.at[slot]).wait()

            z1 = _gelu(_dot(hln_v[r, :], win_v[:, :FH]))
            g = _dot(wsp_v[r, :], z2_v[...])
            bcol = bcol_v[r, :]
            g = g + jnp.tile(bcol, (1, FH // 128))
            y = _dot((z1 * g).astype(BF16), wout_v[...])
            out_v[slot] = (h_v[r, :] + y).astype(BF16)
            pltpu.make_async_copy(out_v.at[slot], out_hbm.at[r], osems.at[slot]).start()
            return 0

        lax.fori_loop(0, NT, p3, 0)
        for s in range(2):
            pltpu.make_async_copy(out_v.at[s], out_hbm.at[pl.ds(0, TM)], osems.at[s]).wait()

    return kernel


def build(TM):
    def fn(A_x, A_wqkv, A_wo, B_x, B_w_in, B_w_sp, B_b_sp, B_w_out):
        x = A_x.reshape(S, D)
        bsp = B_b_sp.reshape(S // 128, 128)
        anyspec = pl.BlockSpec(memory_space=pl.ANY)
        out = pl.pallas_call(
            make_kernel(TM),
            out_shape=jax.ShapeDtypeStruct((S, D), BF16),
            in_specs=[anyspec] * 5 + [pl.BlockSpec(memory_space=pltpu.VMEM), anyspec],
            out_specs=anyspec,
            scratch_shapes=[
                pltpu.VMEM((S, D), BF16), pltpu.VMEM((D, 3 * D), BF16), pltpu.VMEM((D, D), BF16),
                pltpu.VMEM((D, 2 * FH), BF16), pltpu.VMEM((S, S), BF16), pltpu.VMEM((FH, D), BF16),
                pltpu.VMEM((S, D), BF16), pltpu.VMEM((S, D), F32), pltpu.VMEM((S, D), BF16),
                pltpu.VMEM((S, FH), BF16), pltpu.VMEM((4, 128, 128), F32), pltpu.VMEM((8, D), F32),
                pltpu.VMEM((D, D), BF16), pltpu.VMEM((4, 128, 128), BF16),
                pltpu.VMEM((2, TM, D), BF16), pltpu.VMEM((S, 128), F32),
                pltpu.SemaphoreType.DMA((6,)), pltpu.SemaphoreType.DMA((2,)),
            ],
            compiler_params=pltpu.CompilerParams(vmem_limit_bytes=100 * 1024 * 1024),
        )(x, A_wqkv, A_wo, B_w_in, B_w_sp, bsp, B_w_out)
        return out.reshape(1, S, D)
    return fn


pallas_sequential_preLN__linear_attn_block__mixer_gmlp__prompt_kernel = jax.jit(build(512))
```

```python
import jax
import jax.numpy as jnp
import numpy as np
from jax import lax
import jax.experimental.pallas as pl
import jax.experimental.pallas.tpu as pltpu

S, D, H, DH, FH = 2048, 512, 32, 16, 896
EPS = 1e-5
F32, BF16, U32 = jnp.float32, jnp.bfloat16, jnp.uint32
R = 512
NT = S // R
R2 = R // 2
CH = 32


def _ln(x):
    m = jnp.mean(x, axis=-1, keepdims=True)
    d = x - m
    v = jnp.mean(d * d, axis=-1, keepdims=True)
    return d * lax.rsqrt(v + EPS)


def _phi(t):
    return jnp.where(t > 0, t + 1.0, jnp.exp(t)) + 1e-6


def _gelu(x):
    c = float(np.sqrt(2.0 / np.pi))
    hx = 0.5 * x
    u = x * (c + (c * 0.044715) * (x * x))
    return hx * jnp.tanh(u) + hx


def _dot(a, b):
    return jnp.dot(a, b, preferred_element_type=F32)


def _pk(x):
    return pltpu.bitcast(x.astype(BF16), U32)


def _upk(x):
    return pltpu.bitcast(x, BF16)


def _rcp(d):
    r = pl.reciprocal(d, approx=True)
    return r * (2.0 - d * r)


def c128(n):
    return slice(n * 128, (n + 1) * 128)


_PROG = (
    ('start', 'x0a', 'wk0'), ('wait', 'x0a'), ('start', 'wk1'), ('LX', 0, 0, 2), ('wait', 'wk0'),
    ('start', 'x0b'), ('K', 0, 0, 0, 2), ('K', 0, 1, 0, 2), ('wait', 'wk1'), ('start', 'x1'),
    ('K', 0, 2, 0, 2), ('XT', 0, 0, 2), ('K', 0, 3, 0, 2), ('wait', 'x0b'), ('start', 'wq'),
    ('start', 'x2!', 'x3!', 'wv!', 'wo!', 'win2!', 'b!'), ('LX', 0, 1, 2), ('ATH', 0, 0, 0),
    ('ATH', 0, 1, 0), ('XT', 0, 1, 2), ('K', 0, 0, 1, 2), ('K', 0, 1, 1, 2), ('K', 0, 2, 1, 2),
    ('K', 0, 3, 1, 2), ('ATH', 0, 0, 1), ('ATH', 0, 1, 1), ('wait', 'x1', 'wq'), ('LX', 1, 0, 2),
    ('Q', 0, 0), ('Q', 0, 1), ('LX', 1, 1, 2), ('XT', 1), ('Q', 0, 2), ('Q', 0, 3), ('K', 1, 0),
    ('K', 1, 1), ('K', 1, 2), ('K', 1, 3), ('AT', 1, 1), ('AT', 1, 2), ('AT', 1, 3),
    ('wait', 'x2', 'x3'), ('start', 's0', 's1', 's2', 's3', 'win1', 'wout'), ('AT', 1, 0),
    ('LX', 2, 0, 2), ('Q', 1, 0), ('Q', 1, 1), ('LX', 2, 1, 2), ('XT', 2), ('Q', 1, 2), ('Q', 1, 3),
    ('K', 2, 0), ('K', 2, 1), ('LX', 3), ('K', 2, 2), ('K', 3, 1), ('K', 2, 3), ('XT', 3),
    ('K', 3, 0), ('K', 3, 2), ('K', 3, 3), ('ZR',), ('ZM',), ('DX', 0), ('AT', 2, 0), ('AT', 2, 1),
    ('AT', 2, 2), ('AT', 2, 3), ('AT', 3, 0), ('AT', 3, 1), ('AT', 3, 2), ('AT', 3, 3),
    ('wait', 'wv', 'wo', 'win2', 'b'), ('Q', 3, 0), ('DN', 1), ('KV', 0), ('KV', 1), ('KV', 2),
    ('KV', 3), ('Q', 3, 1), ('WP', 0), ('WP', 1), ('WP', 2), ('WP', 3), ('Q', 3, 2), ('BC',),
    ('Q', 3, 3), ('O', 0, 0), ('O', 0, 1), ('O', 0, 2), ('O', 0, 3), ('Q', 2, 0), ('LH', 0, 0, 2),
    ('Q', 2, 1), ('LH', 0, 1, 2), ('Z2', 0, None, 0, 4), ('Z2', 0, None, 1, 4), ('LZ', 0, 0, 4),
    ('Q', 2, 2), ('Z2', 0, None, 2, 4), ('LZ', 0, 1, 4), ('Z2', 0, None, 3, 4), ('LZ', 0, 2, 4),
    ('Q', 2, 3), ('LZ', 0, 3, 4), ('O', 1, 0), ('O', 1, 1), ('O', 1, 2), ('O', 1, 3),
    ('wait', 's0', 's1', 's2', 's3', 'win1', 'wout'), ('G', 0, 0), ('LH', 1), ('G', 0, 1),
    ('DX', 2), ('G', 0, 2), ('G', 0, 3), ('Z2', 1, None, 0, 4), ('LZ', 1, 0, 4),
    ('Z2', 1, None, 1, 4), ('G', 0, 4), ('LZ', 1, 1, 4), ('Z2', 1, None, 2, 4), ('G', 0, 5),
    ('LZ', 1, 2, 4), ('Z2', 1, None, 3, 4), ('G', 0, 6), ('O', 2, 1), ('O', 2, 2), ('O', 2, 3),
    ('O', 2, 0), ('LZ', 1, 3, 4), ('G', 1, 0), ('LH', 2), ('G', 1, 1), ('DX', 3), ('G', 1, 2),
    ('Z2', 2, None, 0, 4), ('G', 1, 3), ('LZ', 2, 0, 4), ('Z2', 2, None, 1, 4), ('G', 1, 4),
    ('LZ', 2, 1, 4), ('Z2', 2, None, 2, 4), ('G', 1, 5), ('LZ', 2, 2, 4), ('Z2', 2, None, 3, 4),
    ('G', 1, 6), ('LZ', 2, 3, 4), ('O', 3, 0), ('O', 3, 1), ('O', 3, 2), ('O', 3, 3), ('G', 2, 0),
    ('LH', 3), ('G', 2, 1), ('G', 2, 2), ('Z2', 3, None, 0, 4), ('G', 2, 3), ('LZ', 3, 0, 4),
    ('Z2', 3, None, 1, 4), ('G', 2, 4), ('LZ', 3, 1, 4), ('Z2', 3, None, 2, 4), ('G', 2, 5),
    ('LZ', 3, 2, 4), ('Z2', 3, None, 3, 4), ('G', 2, 6), ('LZ', 3, 3, 4), ('Z1', 0), ('GL', 0),
    ('Z1', 1), ('Y', 0), ('GL', 1), ('Z1', 2), ('Y', 1), ('GL', 2), ('Z1', 3), ('Y', 2), ('GL', 3),
    ('Y', 3, 0, 4), ('Y', 3, 1, 4), ('Y', 3, 2, 4), ('Y', 3, 6, 8), ('Y', 3, 14, 16),
    ('Y', 3, 15, 16),
)


def _kernel(x_hbm, wqkv_hbm, wo_hbm, win_hbm, wsp_hbm, bsp_hbm, wout_hbm, out_hbm,
           x_v, wqkv_v, wo_v, win_v, wsp_v, wout_v,
           xl_v, xt_v, pk_v, pq_v, h_v, hl_v, zs_v, z2_v, at_v, wp_v, zm_v, g_v, bc_v, out_v,
           kv_v, bsp_v, z1_v, u_v, zr_v,
           xsem, wsem, ssem, osem):
    def rows(i):
        return slice(i * R, (i + 1) * R)

    def rows2(i):
        return slice(i * R2, (i + 1) * R2)

    def part(lo, n, p, np_):
        return slice(lo + p * n // np_, lo + (p + 1) * n // np_)

    def half(r):
        return slice(r.start // 2, r.stop // 2)

    cp = {}
    def reg(name, src, dst, sem):
        cp[name] = pltpu.make_async_copy(src, dst, sem)
    for i in range(1, NT):
        reg(f'x{i}', x_hbm.at[rows(i)], x_v.at[rows(i)], xsem.at[i])
    for p in range(2):
        r = part(0, R, p, 2)
        reg(f'x0{"ab"[p]}', x_hbm.at[r], x_v.at[r], xsem.at[4 * p])
    for k, nm in ((0, 'q'), (2, 'v')):
        cs = slice(k * D, (k + 1) * D)
        reg('w' + nm, wqkv_hbm.at[:, cs], wqkv_v.at[:, cs], wsem.at[k])
    for p in range(2):
        cs = slice(D + p * 256, D + (p + 1) * 256)
        reg(f'wk{p}', wqkv_hbm.at[:, cs], wqkv_v.at[:, cs], wsem.at[8 + p])
    reg('wo', wo_hbm, wo_v, wsem.at[3])
    reg('win2', win_hbm.at[:, FH:], win_v.at[:, FH:], wsem.at[4])
    reg('win1', win_hbm.at[:, :FH], win_v.at[:, :FH], wsem.at[5])
    reg('wout', wout_hbm, wout_v, wsem.at[6])
    reg('b', bsp_hbm, bsp_v, wsem.at[7])
    for j in range(NT):
        reg(f's{j}', wsp_hbm.at[:, rows(j)], wsp_v.at[j], ssem.at[j])
    zacc = [None] * 4
    ocps = []

    def start(*names):
        for n in names:
            if n.endswith('!'):
                cp[n[:-1]].start(priority=1)
            else:
                cp[n].start()

    def wait(*names):
        for n in names:
            cp[n].wait()

    def chunks(lo, p, np_, ch):
        nc = R // ch
        return [slice(lo + c * ch, lo + (c + 1) * ch) for c in range(p * nc // np_, (p + 1) * nc // np_)]

    def LX(i, p=0, np_=1):
        for r in chunks(i * R, p, np_, CH):
            xl_v[half(r), :] = _pk(_ln(x_v[r, :].astype(F32)))

    def XT(i, p=0, np_=1):
        r = part(0, R, p, np_)
        xl = _upk(xl_v[i * R2 + r.start // 2:i * R2 + r.stop // 2, :])
        xt_v[i % 2, :, r] = pltpu.bitcast(xl.T, U32)

    def K(i, n, p=0, np_=1):
        r = part(i * R, R, p, np_)
        k = _dot(_upk(xl_v[half(r), :]), wqkv_v[:, D + n * 128:D + (n + 1) * 128])
        pk = _phi(k)
        m = r.stop - r.start
        pk_v[i % 2, n, half(part(0, R, p, np_)), :] = _pk(pk)
        zs = jnp.sum(pk.reshape(m // 8, 8, 128), axis=0)
        zacc[n] = zs if zacc[n] is None else zacc[n] + zs

    def Q(i, n):
        q = _dot(_upk(xl_v[rows2(i), :]), wqkv_v[:, n * 128:(n + 1) * 128])
        pq_v[rows2(i), c128(n)] = _pk(_phi(q))

    def AT(i, n):
        r = _dot(_upk(xt_v[i % 2]), _upk(pk_v[i % 2, n]))
        if i == 0:
            at_v[:, c128(n)] = r
        else:
            at_v[:, c128(n)] += r

    def ATH(i, n2, p):
        r = part(0, R, p, 2)
        w = jnp.concatenate([_upk(pk_v[i % 2, n, half(r), :]) for n in (2 * n2, 2 * n2 + 1)], axis=1)
        res = _dot(_upk(xt_v[i % 2, :, r]), w)
        cs = slice(n2 * 256, (n2 + 1) * 256)
        if i == 0 and p == 0:
            at_v[:, cs] = res
        else:
            at_v[:, cs] += res

    def _mask():
        ri = lax.broadcasted_iota(jnp.int32, (128, 128), 0) // DH
        ci = lax.broadcasted_iota(jnp.int32, (128, 128), 1) // DH
        return ri == ci

    def KV(b):
        kvb = lax.dot_general(at_v[:, c128(b)].astype(BF16), wqkv_v[:, 2 * D + b * 128:2 * D + (b + 1) * 128],
                              (((0,), (0,)), ((), ())), preferred_element_type=F32)
        kv_v[b] = _pk(jnp.where(_mask(), kvb, 0.0))

    def WP(b):
        wp_v[c128(b), :] = _dot(_upk(kv_v[b]), wo_v[c128(b), :]).astype(BF16)

    def ZM():
        for b in range(4):
            zrow = jnp.sum(zacc[b], axis=0, keepdims=True)
            zm_v[b] = jnp.where(_mask(), jnp.broadcast_to(zrow, (128, 128)), 0.0).astype(BF16)

    def BC():
        brow = bsp_v[...].astype(F32)
        for j in range(S // 128):
            bc_v[j * 128:(j + 1) * 128, :] = jnp.broadcast_to(brow[j:j + 1, :], (128, 128)).T

    def DN(i, b=None):
        for b in (range(4) if b is None else [b]):
            pqb = _upk(pq_v[rows2(i), c128(b)])
            den = lax.dot_general(pqb, zm_v[b], (((1,), (1,)), ((), ())), preferred_element_type=F32)
            pq_v[rows2(i), c128(b)] = _pk(pqb.astype(F32) * _rcp(den + 1e-6))

    def ZR():
        for b in range(4):
            zr_v[b] = jnp.broadcast_to(jnp.sum(zacc[b], axis=0, keepdims=True), (8, 128)).astype(BF16).astype(F32)

    def DX(i):
        for b in range(4):
            pq = _upk(pq_v[rows2(i), c128(b)]).astype(F32)
            t = pq * jnp.tile(zr_v[b], (R // 8, 1))
            for sh in (1, 2, 4, 8):
                t = t + pltpu.roll(t, sh, 1)
            lane = lax.broadcasted_iota(jnp.int32, t.shape, 1)
            den = jnp.take_along_axis(t, lane | (DH - 1), axis=1)
            pq_v[rows2(i), c128(b)] = _pk(pq * _rcp(den + 1e-6))

    def O(i, n=None, p=0, np_=1):
        r = part(0, R, p, np_)
        cs = slice(0, D) if n is None else c128(n)
        rr = slice(i * R + r.start, i * R + r.stop)
        res = _dot(_upk(pq_v[half(rr), :]), wp_v[:, cs])
        h_v[rr, cs] = x_v[rr, cs].astype(F32) + res

    def LH(i, p=0, np_=1):
        for r in chunks(i * R, p, np_, CH):
            hl_v[half(r), :] = _pk(_ln(h_v[r, :]))

    def Z2(i, n=None, p=0, np_=1):
        r = part(0, R, p, np_)
        rr = slice(i * R + r.start, i * R + r.stop)
        cs = slice(0, FH) if n is None else c128(n)
        res = _dot(_upk(hl_v[half(rr), :]), win_v[:, FH + cs.start:FH + cs.stop])
        zs_v[r, cs] = _gelu(res)

    def LZ(i, p=0, np_=1):
        for r in chunks(0, p, np_, CH):
            rr = slice(i * R + r.start, i * R + r.stop)
            z2_v[half(rr), :] = _pk(_ln(zs_v[r, :]))

    def G(j, n, p=0, np_=1):
        rs = part(0, S, p, np_)
        r = _dot(wsp_v[j, rs, :], _upk(z2_v[rows2(j), c128(n)]))
        if j == 0:
            g_v[rs, c128(n)] = r + bc_v[rs, :]
        else:
            g_v[rs, c128(n)] += r

    def Z1(i, n=None):
        cs = slice(0, FH) if n is None else c128(n)
        z1_v[i % 2, :, cs] = _gelu(_dot(_upk(hl_v[rows2(i), :]), win_v[:, cs]))

    def GL(i, n=None):
        cs = slice(0, FH) if n is None else c128(n)
        g = g_v[rows(i), cs] + _dot(wsp_v[NT - 1, rows(i), :], _upk(z2_v[rows2(NT - 1), cs]))
        u_v[i % 2, :, cs] = _pk(z1_v[i % 2, :, cs] * g)

    def Y(i, p=0, np_=1):
        rl = part(0, R, p, np_)
        r = slice(i * R + rl.start, i * R + rl.stop)
        y = _dot(_upk(u_v[i % 2, half(rl), :]), wout_v[...])
        out_v[r, :] = (h_v[r, :] + y).astype(BF16)
        c = pltpu.make_async_copy(out_v.at[r], out_hbm.at[r], osem.at[len(ocps)])
        c.start()
        ocps.append(c)

    env = dict(start=start, wait=wait, LX=LX, XT=XT, K=K, Q=Q, AT=AT, ATH=ATH, KV=KV, WP=WP, ZM=ZM, BC=BC,
               DN=DN, DX=DX, ZR=ZR, O=O, LH=LH, Z2=Z2, LZ=LZ, G=G, Z1=Z1, GL=GL, Y=Y)
    for tok in _PROG:
        env[tok[0]](*tok[1:])
    for c in ocps:
        c.wait()


@jax.jit
def pallas_sequential_preLN__linear_attn_block__mixer_gmlp__prompt_kernel(
    A_x: jax.Array,
    A_wqkv: jax.Array,
    A_wo: jax.Array,
    B_x: jax.Array,
    B_w_in: jax.Array,
    B_w_sp: jax.Array,
    B_b_sp: jax.Array,
    B_w_out: jax.Array,
):
    del B_x
    x = A_x.reshape(S, D)
    bsp = B_b_sp.reshape(S // 128, 128)
    anyspec = pl.BlockSpec(memory_space=pl.ANY)
    out = pl.pallas_call(
        _kernel,
        out_shape=jax.ShapeDtypeStruct((S, D), BF16),
        in_specs=[anyspec] * 7,
        out_specs=anyspec,
        scratch_shapes=[
            pltpu.VMEM((S, D), BF16), pltpu.VMEM((D, 3 * D), BF16), pltpu.VMEM((D, D), BF16),
            pltpu.VMEM((D, 2 * FH), BF16), pltpu.VMEM((NT, S, R), BF16), pltpu.VMEM((FH, D), BF16),
            pltpu.VMEM((S // 2, D), U32),
            pltpu.VMEM((2, D // 2, R), U32),
            pltpu.VMEM((2, 4, R2, 128), U32),
            pltpu.VMEM((S // 2, D), U32),
            pltpu.VMEM((S, D), F32),
            pltpu.VMEM((S // 2, D), U32),
            pltpu.VMEM((R, FH), F32),
            pltpu.VMEM((S // 2, FH), U32),
            pltpu.VMEM((D, D), F32),
            pltpu.VMEM((D, D), BF16),
            pltpu.VMEM((4, 128, 128), BF16),
            pltpu.VMEM((S, FH), F32),
            pltpu.VMEM((S, 128), F32),
            pltpu.VMEM((S, D), BF16),
            pltpu.VMEM((4, 64, 128), U32),
            pltpu.VMEM((S // 128, 128), BF16),
            pltpu.VMEM((2, R, FH), F32),
            pltpu.VMEM((2, R2, FH), U32),
            pltpu.VMEM((4, 8, 128), F32),
            pltpu.SemaphoreType.DMA((5,)), pltpu.SemaphoreType.DMA((10,)),
            pltpu.SemaphoreType.DMA((NT,)), pltpu.SemaphoreType.DMA((9,)),
        ],
        compiler_params=pltpu.CompilerParams(vmem_limit_bytes=100 * 1024 * 1024),
    )(x, A_wqkv, A_wo, B_w_in, B_w_sp, bsp, B_w_out)
    return out.reshape(1, S, D)
```
